```python
import os as _os
_os.environ.setdefault("JAX_PLATFORMS", "cpu")
import jax
import jax.numpy as jnp

def _softmax(x, axis=-1):
    return jax.nn.softmax(x, axis=axis)
def _gelu(x):
    return jax.nn.gelu(x, approximate=True)
def _silu(x):
    return jax.nn.silu(x)
def _sigmoid(x):
    return jax.nn.sigmoid(x)
def _layernorm(x, axis=-1, eps=1e-5):
    m = jnp.mean(x, axis=axis, keepdims=True)
    v = jnp.var(x, axis=axis, keepdims=True)
    return (x - m) / jnp.sqrt(v + eps)
def _scatter_add(tgt, idx, src, axis=0):
    return tgt.at[idx].add(src)
def _segment_sum(src, seg, n):
    return jax.ops.segment_sum(src, seg, n)
class _Rng:
    def __init__(self, key):
        self._k = key
    def _next(self):
        self._k, sub = jax.random.split(self._k)
        return sub
    def normal(self, shape):
        return jax.random.normal(self._next(), shape, dtype=jnp.bfloat16)
    def randint(self, lo, hi, shape):
        return jax.random.randint(self._next(), shape, lo, hi, dtype=jnp.int32)
    def uniform(self, shape, lo=0.0, hi=1.0):
        return jax.random.uniform(self._next(), shape, jnp.bfloat16, lo, hi)
    def permutation(self, n):
        return jax.random.permutation(self._next(), n)


kernel_name = 'sequential_preLN__sliding_local_dilated__dense_activation_mish__prompt'

def setup_inputs():
    _rng = _Rng(jax.random.key(int.from_bytes(__import__("os").urandom(4), "little")))
    _w = (lambda a: (lambda t: t.astype(jnp.bfloat16) if jnp.issubdtype(t.dtype, jnp.floating) else t)(jnp.asarray(a)))
    def _A_setup():
        B, S, D = 1, 2048, 512
        return {
            "x": _w((lambda *s: _rng.normal(s) * 0.05)(B, S, D)),
            "wqkv": _w((lambda *s: _rng.normal(s) * 0.05)(D, 3 * D)),
            "wo": _w((lambda *s: _rng.normal(s) * 0.05)(D, D)),
        }
    _A_in = _A_setup()

    def _B_setup():
        B, S, D, F = 1, 2048, 512, 1376
        return {
            "x": _w((lambda *s: _rng.normal(s) * 0.05)(B, S, D)),
            "w1": _w((lambda *s: _rng.normal(s) * 1.6)(D, F) * (D ** -0.5)),
            "b1": _w((lambda *s: _rng.normal(s) * 0.1)(F)),
            "w2": _w((lambda *s: _rng.normal(s) * 0.1)(F, D) * (F ** -0.5)),
        }
    _B_in = _B_setup()

    return {
        "A_x": _A_in["x"],
        "A_wqkv": _A_in["wqkv"],
        "A_wo": _A_in["wo"],
        "B_x": _B_in["x"],
        "B_w1": _B_in["w1"],
        "B_b1": _B_in["b1"],
        "B_w2": _B_in["w2"],
    }

def reference(A_x, A_wqkv, A_wo, B_x, B_w1, B_b1, B_w2):
    def _A_ref(x, wqkv, wo):
        B, S, D = x.shape
        H = 32; Dh = D // H
        W, dil = 8, 2
        qkv = (lambda x, *d: x.transpose(*d))((x @ wqkv).reshape(B, S, 3, H, Dh), 2, 0, 3, 1, 4)
        q, k, v = qkv[0], qkv[1], qkv[2]
        scale = Dh ** -0.5
        pos = jnp.arange(S)
        off = jnp.arange(W) * dil
        idx = pos[:, None] - off[None, :]
        mask = idx >= 0
        idx_c = jnp.where(mask, idx, 0).reshape(-1)
        kg = k[:, :, idx_c, :].reshape(B, H, S, W, Dh)
        vg = v[:, :, idx_c, :].reshape(B, H, S, W, Dh)
        logits = jnp.einsum("bhsd,bhswd->bhsw", q, kg) * scale
        logits = jnp.where(mask[None, None, :, :], logits, -1e9)
        attn = _softmax(logits, axis=-1)
        o = jnp.einsum("bhsw,bhswd->bhsd", attn, vg)
        return (lambda x, *d: x.transpose(*d))(o, 0, 2, 1, 3).reshape(B, S, D) @ wo

    def _B_ref(x, w1, b1, w2):
        h = jnp.einsum("bsd,df->bsf", x, w1) + b1
        sp = jnp.log1p(jnp.exp(-jnp.abs(h))) + jnp.where(h > 0, h, jnp.zeros_like(h))
        act = h * jnp.tanh(sp)
        return jnp.einsum("bsf,fd->bsd", act, w2)

    x = A_x
    h = x + _A_ref(_layernorm(x, axis=-1), A_wqkv, A_wo)
    h2 = h + _B_ref(_layernorm(h, axis=-1), B_w1, B_b1, B_w2)
    return h2
```

```python
import functools

import jax
import jax.numpy as jnp
from jax.experimental import pallas as pl
from jax.experimental.pallas import tpu as pltpu

S, D, H, DH, W, DIL, F = 2048, 512, 32, 16, 8, 2, 1376
T = 512
HALO = 16
ST = 17
SCALE = DH ** -0.5
LOG2E = 1.4426950408889634
NEG = -1e9 / SCALE
CHAIN = 3
f32, bf16, i32 = jnp.float32, jnp.bfloat16, jnp.int32


def _ln(x):
    m = jnp.mean(x, axis=-1, keepdims=True)
    xc = x - m
    v = jnp.mean(xc * xc, axis=-1, keepdims=True)
    return xc * jax.lax.rsqrt(v + 1e-5)


def _mish(h):
    e = jnp.exp(jnp.minimum(h, 30.0))
    n = e * (e + 2.0)
    return h * n * pl.reciprocal(n + 2.0, approx=True)


def _dot_nn(a, b):
    return jnp.dot(a, b, preferred_element_type=f32)


def _dot_nt(a, b):
    return jax.lax.dot_general(a, b, (((1,), (1,)), ((), ())), preferred_element_type=f32)


def _kernel(x_hbm, wqkv_hbm, wo_hbm, w1t_hbm, b1_hbm, w2_hbm, o_hbm,
            x_v, wraw, woraw, wt, wo_v, w1t_v, b1_v, w2_v, o_v,
            qkv0, qkv1, a_s, s32, h_s, hn_s, isem, osem):
    cx = [pltpu.make_async_copy(x_hbm.at[pl.ds(i * T, T), :], x_v.at[pl.ds(i * T, T), :], isem.at[i])
          for i in range(4)]
    cw = [pltpu.make_async_copy(wqkv_hbm.at[:, pl.ds(p * D, D)], wraw.at[:, pl.ds(p * D, D)], isem.at[4 + p])
          for p in range(3)]
    cwo = pltpu.make_async_copy(wo_hbm, woraw, isem.at[7])
    cw1 = pltpu.make_async_copy(w1t_hbm, w1t_v, isem.at[8])
    cb1 = pltpu.make_async_copy(b1_hbm, b1_v, isem.at[9])
    cw2 = pltpu.make_async_copy(w2_hbm, w2_v, isem.at[10])
    for c in (cw[1], cx[0], cw[2], cw[0], cx[1], cwo, cx[2], cw1, cb1, cw2, cx[3]):
        c.start()

    out_copies = []

    def put_heads(kt, i, rows):
        for m in range(8):
            hd = i * 8 + m
            s32[kt, hd * ST:hd * ST + DH, :] = rows[m * DH:(m + 1) * DH, :]

    def regroup(dst, base):
        for kt in range(4):
            for d in range(DH):
                for h0 in (0, 16):
                    lo = s32[kt, pl.ds(h0 * ST + d, 8, stride=ST), :]
                    hi = s32[kt, pl.ds((h0 + 8) * ST + d, 8, stride=ST), :]
                    r = base + d * H + h0
                    dst[r:r + 16, kt * 128:(kt + 1) * 128] = jnp.concatenate([lo, hi], axis=0).astype(bf16)

    def perm_w(p):
        for i in range(4):
            wT = wraw[:, p * D + i * 128:p * D + (i + 1) * 128].astype(f32).T
            for kt in range(4):
                put_heads(kt, i, wT[:, kt * 128:(kt + 1) * 128])
        regroup(wt, p * D)

    def perm_wo():
        for kt in range(4):
            for i in range(4):
                put_heads(kt, i, woraw[i * 128:(i + 1) * 128, kt * 128:(kt + 1) * 128].astype(f32))
        regroup(wo_v, 0)

    def proj(dst, p, xn, r0=0, tiles=(0, 4), first=False):
        j0, j1 = tiles
        n = xn.shape[0]
        y = _dot_nt(xn, wt[p * D + j0 * 128:p * D + j1 * 128, :])
        for j in range(j0, j1):
            yj = y[:, (j - j0) * 128:(j - j0 + 1) * 128]
            dst[p, j, HALO + r0:HALO + r0 + n, :] = yj
            if first and p == 1:
                dst[p, j, 0:HALO, :] = jnp.zeros((HALO, 128), f32)
            if first and p == 2:
                dst[p, j, 0:HALO, :] = jnp.broadcast_to(yj[0:1, :], (HALO, 128))

    def halo(src, dst):
        for p in (1, 2):
            for j in range(4):
                dst[p, j, 0:HALO, :] = src[p, j, T:T + HALO, :]

    hist = []

    def attention(buf, r0=0, n=T, first=False):
        for r in range(r0, r0 + n, 8):
            q = [buf[0, j, HALO + r:HALO + r + 8, :] for j in range(4)]
            if len(hist) >= CHAIN:
                z = jax.lax.shift_right_logical(pltpu.bitcast(hist[-CHAIN], i32), 31)
                q[0] = pltpu.bitcast(pltpu.bitcast(q[0], i32) | z, f32)
            ls = []
            for w in range(W):
                t0 = HALO + r - DIL * w
                p = None
                for j in range(4):
                    t = q[j] * buf[1, j, t0:t0 + 8, :]
                    p = t if p is None else p + t
                p = p + pltpu.roll(p, 64, 1)
                p = p + pltpu.roll(p, 32, 1)
                if first and r - DIL * w < 0:
                    rows = jax.lax.broadcasted_iota(i32, (8, 128), 0) + r
                    p = jnp.where(rows >= DIL * w, p, NEG)
                ls.append(p)
            m = functools.reduce(jnp.maximum, ls)
            es = [jnp.exp2((l - m) * (SCALE * LOG2E)) for l in ls]
            rinv = pl.reciprocal(functools.reduce(jnp.add, es), approx=True)
            hist.append(rinv)
            outs = []
            for j in range(4):
                acc = None
                for w in range(W):
                    t0 = HALO + r - DIL * w
                    t = es[w] * buf[2, j, t0:t0 + 8, :]
                    acc = t if acc is None else acc + t
                outs.append(acc * rinv)
            o = jnp.concatenate(outs, axis=1)
            if r % 16 == 0:
                prev = o
            else:
                a_s[r - 8:r + 8, :] = jnp.concatenate([prev, o], axis=0).astype(bf16)

    def out_proj(xrows, r0=0, n=T):
        return xrows.astype(f32) + _dot_nn(a_s[r0:r0 + n, :], wo_v[...])

    def mlp(h, hn, g0, sem_idx):
        n = h.shape[0]
        pre = _dot_nt(hn, w1t_v[...]) + b1_v[...].astype(f32).reshape(1, F)
        y = _dot_nn(_mish(pre).astype(bf16), w2_v[...])
        o_v[pl.ds(g0, n), :] = (h + y).astype(o_v.dtype)
        pltpu.make_async_copy(o_v.at[pl.ds(g0, n), :], o_hbm.at[pl.ds(g0, n), :], osem.at[sem_idx]).start()

    def ln1(rows):
        return _ln(rows.astype(f32)).astype(bf16)

    cw[1].wait()
    perm_w(1)
    cx[0].wait()
    xn0 = ln1(x_v[0:T, :])
    proj(qkv0, 1, xn0, tiles=(0, 2), first=True)
    cw[2].wait()
    proj(qkv0, 1, xn0, tiles=(2, 4), first=True)
    perm_w(2)
    cw[0].wait()
    proj(qkv0, 2, xn0, first=True)
    perm_w(0)
    cx[1].wait()
    cwo.wait()
    Q = T // 4
    xn1 = None
    for c in range(4):
        proj(qkv0, 0, xn0[c * Q:(c + 1) * Q, :], r0=c * Q)
        if c == 0:
            perm_wo()
            xn1 = ln1(x_v[T:2 * T, :])
        attention(qkv0, c * Q, Q, first=True)
    halo(qkv0, qkv1)
    for p in (1, 2, 0):
        proj(qkv1, p, xn1)
    hq = []
    for c in range(4):
        hq.append(out_proj(x_v[c * Q:(c + 1) * Q, :], c * Q, Q))
        if c >= 1:
            hn_s[(c - 1) * Q:c * Q, :] = _ln(hq[c - 1]).astype(bf16)
    hn_s[3 * Q:4 * Q, :] = _ln(hq[3]).astype(bf16)
    h_s[...] = jnp.concatenate(hq, axis=0)
    for c in (cw1, cb1, cw2, cx[2], cx[3]):
        c.wait()

    def body(i, carry):
        g0 = pl.multiple_of(i * T, T)
        g1 = pl.multiple_of((i + 1) * T, T)
        g2 = pl.multiple_of((i + 2) * T, T)
        mlp(h_s[...], hn_s[...], g0, i)
        hist.clear()
        attention(qkv1)
        hist.clear()
        h = out_proj(x_v[pl.ds(g1, T), :])
        h_s[...] = h
        halo(qkv1, qkv1)
        xn = ln1(x_v[pl.ds(g2, T), :])
        for p in (1, 2, 0):
            proj(qkv1, p, xn)
        hn_s[...] = _ln(h).astype(bf16)
        return carry

    jax.lax.fori_loop(0, 2, body, 0)

    mlp(h_s[...], hn_s[...], 2 * T, 2)
    attention(qkv1)
    Hf = T // 2
    h3 = [out_proj(x_v[3 * T + c * Hf:3 * T + (c + 1) * Hf, :], c * Hf, Hf) for c in range(2)]
    hn3 = [_ln(h).astype(bf16) for h in h3]
    mlp(h3[0], hn3[0], 3 * T, 3)
    for c in range(2):
        mlp(h3[1][c * Q:(c + 1) * Q, :], hn3[1][c * Q:(c + 1) * Q, :], 3 * T + Hf + c * Q, 4 + c)

    for sem_idx, (g0, n) in enumerate(((0, T), (T, T), (2 * T, T), (3 * T, Hf), (3 * T + Hf, Q), (3 * T + Hf + Q, Q))):
        pltpu.make_async_copy(o_v.at[pl.ds(g0, n), :], o_hbm.at[pl.ds(g0, n), :], osem.at[sem_idx]).wait()


@jax.jit
def pallas_sequential_preLN__sliding_local_dilated__dense_activation_mish__prompt_kernel(
    A_x: jax.Array,
    A_wqkv: jax.Array,
    A_wo: jax.Array,
    B_x: jax.Array,
    B_w1: jax.Array,
    B_b1: jax.Array,
    B_w2: jax.Array,
):
    del B_x
    hbm = pl.BlockSpec(memory_space=pltpu.HBM)
    out = pl.pallas_call(
        _kernel,
        out_shape=jax.ShapeDtypeStruct((S, D), bf16),
        in_specs=[hbm] * 6,
        out_specs=hbm,
        scratch_shapes=[
            pltpu.VMEM((S, D), bf16),
            pltpu.VMEM((D, 3 * D), bf16),
            pltpu.VMEM((D, D), bf16),
            pltpu.VMEM((3 * D, D), bf16),
            pltpu.VMEM((D, D), bf16),
            pltpu.VMEM((F, D), bf16),
            pltpu.VMEM((F,), bf16),
            pltpu.VMEM((F, D), bf16),
            pltpu.VMEM((S, D), bf16),
            pltpu.VMEM((3, 4, T + HALO, 128), f32),
            pltpu.VMEM((3, 4, T + HALO, 128), f32),
            pltpu.VMEM((T, D), bf16),
            pltpu.VMEM((4, H * ST, 128), f32),
            pltpu.VMEM((T, D), f32),
            pltpu.VMEM((T, D), bf16),
            pltpu.SemaphoreType.DMA((11,)),
            pltpu.SemaphoreType.DMA((6,)),
        ],
        compiler_params=pltpu.CompilerParams(
            vmem_limit_bytes=100 * 1024 * 1024,
            flags={"XLA_TPU_EVENLY_DISTRIBUTE_CRITICAL_NODES": True},
            disable_semaphore_checks=True,
        ),
    )(A_x.reshape(S, D), A_wqkv, A_wo, B_w1.T, B_b1, B_w2)
    return out.reshape(1, S, D)
```

```python
import functools

import jax
import jax.numpy as jnp
from jax.experimental import pallas as pl
from jax.experimental.pallas import tpu as pltpu

S, D, H, DH, W, DIL, F = 2048, 512, 32, 16, 8, 2, 1376
T = 512
HALO = 16
ST = 17
SCALE = DH ** -0.5
LOG2E = 1.4426950408889634
NEG = -1e9 / SCALE
CHAIN = 3
f32, bf16, i32 = jnp.float32, jnp.bfloat16, jnp.int32


def _ln(x):
    m = jnp.mean(x, axis=-1, keepdims=True)
    xc = x - m
    v = jnp.mean(xc * xc, axis=-1, keepdims=True)
    return xc * jax.lax.rsqrt(v + 1e-5)


def _mish(h):
    e = jnp.exp(jnp.minimum(h, 30.0))
    n = e * (e + 2.0)
    return h * n * pl.reciprocal(n + 2.0, approx=True)


def _dot_nn(a, b):
    return jnp.dot(a, b, preferred_element_type=f32)


def _dot_nt(a, b):
    return jax.lax.dot_general(a, b, (((1,), (1,)), ((), ())), preferred_element_type=f32)


def _kernel(x_hbm, wqkv_hbm, wo_hbm, w1t_hbm, b1_hbm, w2_hbm, o_hbm,
            x_v, wraw, woraw, wt, wo_v, w1t_v, b1_v, w2_v, o_v,
            qkv0, qkv1, a_s, s32, h_s, hn_s, isem, osem):
    cx = [pltpu.make_async_copy(x_hbm.at[pl.ds(i * T, T), :], x_v.at[pl.ds(i * T, T), :], isem.at[i])
          for i in range(4)]
    cw = [pltpu.make_async_copy(wqkv_hbm.at[:, pl.ds(p * D, D)], wraw.at[:, pl.ds(p * D, D)], isem.at[4 + p])
          for p in range(3)]
    cwo = pltpu.make_async_copy(wo_hbm, woraw, isem.at[7])
    cw1 = pltpu.make_async_copy(w1t_hbm, w1t_v, isem.at[8])
    cb1 = pltpu.make_async_copy(b1_hbm, b1_v, isem.at[9])
    cw2 = pltpu.make_async_copy(w2_hbm, w2_v, isem.at[10])
    for c in (cw[1], cx[0], cw[2], cw[0], cx[1], cwo, cx[2], cw1, cb1, cw2, cx[3]):
        c.start()

    def put_heads(kt, i, rows):
        for m in range(8):
            hd = i * 8 + m
            s32[kt, hd * ST:hd * ST + DH, :] = rows[m * DH:(m + 1) * DH, :]

    def regroup(dst, base):
        for kt in range(4):
            for d in range(DH):
                for h0 in (0, 16):
                    lo = s32[kt, pl.ds(h0 * ST + d, 8, stride=ST), :]
                    hi = s32[kt, pl.ds((h0 + 8) * ST + d, 8, stride=ST), :]
                    r = base + d * H + h0
                    dst[r:r + 16, kt * 128:(kt + 1) * 128] = jnp.concatenate([lo, hi], axis=0).astype(bf16)

    def perm_w(p):
        for i in range(4):
            wT = wraw[:, p * D + i * 128:p * D + (i + 1) * 128].astype(f32).T
            for kt in range(4):
                put_heads(kt, i, wT[:, kt * 128:(kt + 1) * 128])
        regroup(wt, p * D)

    def perm_wo():
        for kt in range(4):
            for i in range(4):
                put_heads(kt, i, woraw[i * 128:(i + 1) * 128, kt * 128:(kt + 1) * 128].astype(f32))
        regroup(wo_v, 0)

    def proj(dst, p, xn, r0=0, tiles=(0, 4), first=False):
        j0, j1 = tiles
        n = xn.shape[0]
        y = _dot_nt(xn, wt[p * D + j0 * 128:p * D + j1 * 128, :])
        for j in range(j0, j1):
            yj = y[:, (j - j0) * 128:(j - j0 + 1) * 128]
            dst[p, j, HALO + r0:HALO + r0 + n, :] = yj
            if first and p == 2:
                dst[p, j, 0:HALO, :] = jnp.broadcast_to(yj[0:1, :], (HALO, 128))

    def halo(src, dst):
        for p in (1, 2):
            for j in range(4):
                dst[p, j, 0:HALO, :] = src[p, j, T:T + HALO, :]

    hist = []

    def attention(buf, r0=0, n=T, first=False):
        for r in range(r0, r0 + n, 8):
            q = [buf[0, j, HALO + r:HALO + r + 8, :] for j in range(4)]
            if len(hist) >= CHAIN:
                z = jax.lax.shift_right_logical(pltpu.bitcast(hist[-CHAIN], i32), 31)
                q[0] = pltpu.bitcast(pltpu.bitcast(q[0], i32) | z, f32)
            ls = []
            for w in range(W):
                t0 = HALO + r - DIL * w
                p = None
                for j in range(4):
                    t = q[j] * buf[1, j, t0:t0 + 8, :]
                    p = t if p is None else p + t
                p = p + pltpu.roll(p, 64, 1)
                p = p + pltpu.roll(p, 32, 1)
                if first and r - DIL * w < 0:
                    rows = jax.lax.broadcasted_iota(i32, (8, 128), 0) + r
                    p = jnp.where(rows >= DIL * w, p, NEG)
                ls.append(p)
            m = functools.reduce(jnp.maximum, ls)
            es = [jnp.exp2((l - m) * (SCALE * LOG2E)) for l in ls]
            rinv = pl.reciprocal(functools.reduce(jnp.add, es), approx=True)
            hist.append(rinv)
            outs = []
            for j in range(4):
                acc = None
                for w in range(W):
                    t0 = HALO + r - DIL * w
                    t = es[w] * buf[2, j, t0:t0 + 8, :]
                    acc = t if acc is None else acc + t
                outs.append(acc * rinv)
            o = jnp.concatenate(outs, axis=1)
            if r % 16 == 0:
                prev = o
            else:
                a_s[r - 8:r + 8, :] = jnp.concatenate([prev, o], axis=0).astype(bf16)

    def out_proj(xrows, r0=0, n=T):
        return xrows.astype(f32) + _dot_nn(a_s[r0:r0 + n, :], wo_v[...])

    def mlp(h, hn, g0, sem_idx):
        n = h.shape[0]
        pre = _dot_nt(hn, w1t_v[...]) + b1_v[...].astype(f32).reshape(1, F)
        y = _dot_nn(_mish(pre).astype(bf16), w2_v[...])
        o_v[pl.ds(g0, n), :] = (h + y).astype(o_v.dtype)
        pltpu.make_async_copy(o_v.at[pl.ds(g0, n), :], o_hbm.at[pl.ds(g0, n), :], osem.at[sem_idx]).start()

    def ln1(rows):
        return _ln(rows.astype(f32)).astype(bf16)

    cw[1].wait()
    perm_w(1)
    cs = _dot_nt(jnp.ones((8, D), bf16), wt[D:2 * D, :])[0:1, :]
    cx[0].wait()
    x0 = x_v[0:T, :].astype(f32)
    m0 = jnp.mean(x0, axis=-1, keepdims=True)
    xc0 = x0 - m0
    rs0 = jax.lax.rsqrt(jnp.mean(xc0 * xc0, axis=-1, keepdims=True) + 1e-5)
    xn0 = (xc0 * rs0).astype(bf16)

    def proj_k0(j0, j1):
        y = _dot_nt(x_v[0:T, :], wt[D + j0 * 128:D + j1 * 128, :])
        for j in range(j0, j1):
            yj = y[:, (j - j0) * 128:(j - j0 + 1) * 128]
            qkv0[1, j, HALO:HALO + T, :] = (yj - m0 * cs[:, j * 128:(j + 1) * 128]) * rs0
            qkv0[1, j, 0:HALO, :] = jnp.zeros((HALO, 128), f32)

    proj_k0(0, 2)
    cw[2].wait()
    proj_k0(2, 4)
    perm_w(2)
    cw[0].wait()
    proj(qkv0, 2, xn0, first=True)
    perm_w(0)
    cx[1].wait()
    cwo.wait()
    Q = T // 4
    xn1 = None
    for c in range(4):
        proj(qkv0, 0, xn0[c * Q:(c + 1) * Q, :], r0=c * Q)
        if c == 0:
            perm_wo()
            xn1 = ln1(x_v[T:2 * T, :])
        attention(qkv0, c * Q, Q, first=True)
    halo(qkv0, qkv1)
    for p in (1, 2, 0):
        proj(qkv1, p, xn1)
    hq = []
    for c in range(4):
        hq.append(out_proj(x_v[c * Q:(c + 1) * Q, :], c * Q, Q))
        if c >= 1:
            hn_s[(c - 1) * Q:c * Q, :] = _ln(hq[c - 1]).astype(bf16)
    hn_s[3 * Q:4 * Q, :] = _ln(hq[3]).astype(bf16)
    h_s[...] = jnp.concatenate(hq, axis=0)
    for c in (cw1, cb1, cw2, cx[2], cx[3]):
        c.wait()

    def body(i, carry):
        g0 = pl.multiple_of(i * T, T)
        g1 = pl.multiple_of((i + 1) * T, T)
        g2 = pl.multiple_of((i + 2) * T, T)
        mlp(h_s[...], hn_s[...], g0, i)
        hist.clear()
        attention(qkv1)
        hist.clear()
        h = out_proj(x_v[pl.ds(g1, T), :])
        h_s[...] = h
        halo(qkv1, qkv1)
        xn = ln1(x_v[pl.ds(g2, T), :])
        for p in (1, 2, 0):
            proj(qkv1, p, xn)
        hn_s[...] = _ln(h).astype(bf16)
        return carry

    jax.lax.fori_loop(0, 2, body, 0)

    mlp(h_s[...], hn_s[...], 2 * T, 2)
    attention(qkv1)
    Hf = T // 2
    h3 = [out_proj(x_v[3 * T + c * Hf:3 * T + (c + 1) * Hf, :], c * Hf, Hf) for c in range(2)]
    hn3 = [_ln(h).astype(bf16) for h in h3]
    mlp(h3[0], hn3[0], 3 * T, 3)
    tail = ((0, Q), (Q, Q // 2), (Q + Q // 2, Q // 2))
    for c, (r, n) in enumerate(tail):
        mlp(h3[1][r:r + n, :], hn3[1][r:r + n, :], 3 * T + Hf + r, 4 + c)

    done = [(0, T), (T, T), (2 * T, T), (3 * T, Hf)] + [(3 * T + Hf + r, n) for r, n in tail]
    for sem_idx, (g0, n) in enumerate(done):
        pltpu.make_async_copy(o_v.at[pl.ds(g0, n), :], o_hbm.at[pl.ds(g0, n), :], osem.at[sem_idx]).wait()


@jax.jit
def pallas_sequential_preLN__sliding_local_dilated__dense_activation_mish__prompt_kernel(
    A_x: jax.Array,
    A_wqkv: jax.Array,
    A_wo: jax.Array,
    B_x: jax.Array,
    B_w1: jax.Array,
    B_b1: jax.Array,
    B_w2: jax.Array,
):
    del B_x
    hbm = pl.BlockSpec(memory_space=pltpu.HBM)
    out = pl.pallas_call(
        _kernel,
        out_shape=jax.ShapeDtypeStruct((S, D), bf16),
        in_specs=[hbm] * 6,
        out_specs=hbm,
        scratch_shapes=[
            pltpu.VMEM((S, D), bf16),
            pltpu.VMEM((D, 3 * D), bf16),
            pltpu.VMEM((D, D), bf16),
            pltpu.VMEM((3 * D, D), bf16),
            pltpu.VMEM((D, D), bf16),
            pltpu.VMEM((F, D), bf16),
            pltpu.VMEM((F,), bf16),
            pltpu.VMEM((F, D), bf16),
            pltpu.VMEM((S, D), bf16),
            pltpu.VMEM((3, 4, T + HALO, 128), f32),
            pltpu.VMEM((3, 4, T + HALO, 128), f32),
            pltpu.VMEM((T, D), bf16),
            pltpu.VMEM((4, H * ST, 128), f32),
            pltpu.VMEM((T, D), f32),
            pltpu.VMEM((T, D), bf16),
            pltpu.SemaphoreType.DMA((11,)),
            pltpu.SemaphoreType.DMA((7,)),
        ],
        compiler_params=pltpu.CompilerParams(
            vmem_limit_bytes=100 * 1024 * 1024,
            flags={"XLA_TPU_EVENLY_DISTRIBUTE_CRITICAL_NODES": True},
            disable_semaphore_checks=True,
        ),
    )(A_x.reshape(S, D), A_wqkv, A_wo, B_w1.T, B_b1, B_w2)
    return out.reshape(1, S, D)
```
